```python
import os as _os
_os.environ.setdefault("JAX_PLATFORMS", "cpu")
import jax
import jax.numpy as jnp

def _softmax(x, axis=-1):
    return jax.nn.softmax(x, axis=axis)
def _gelu(x):
    return jax.nn.gelu(x, approximate=True)
def _silu(x):
    return jax.nn.silu(x)
def _sigmoid(x):
    return jax.nn.sigmoid(x)
def _layernorm(x, axis=-1, eps=1e-5):
    m = jnp.mean(x, axis=axis, keepdims=True)
    v = jnp.var(x, axis=axis, keepdims=True)
    return (x - m) / jnp.sqrt(v + eps)
def _scatter_add(tgt, idx, src, axis=0):
    return tgt.at[idx].add(src)
def _segment_sum(src, seg, n):
    return jax.ops.segment_sum(src, seg, n)
class _Rng:
    def __init__(self, key):
        self._k = key
    def _next(self):
        self._k, sub = jax.random.split(self._k)
        return sub
    def normal(self, shape):
        return jax.random.normal(self._next(), shape, dtype=jnp.bfloat16)
    def randint(self, lo, hi, shape):
        return jax.random.randint(self._next(), shape, lo, hi, dtype=jnp.int32)
    def uniform(self, shape, lo=0.0, hi=1.0):
        return jax.random.uniform(self._next(), shape, jnp.bfloat16, lo, hi)
    def permutation(self, n):
        return jax.random.permutation(self._next(), n)


kernel_name = 'concat_heads__gqa_block_cached__mha_block_cached__near_ridge'

def setup_inputs():
    _rng = _Rng(jax.random.key(int.from_bytes(__import__("os").urandom(4), "little")))
    _w = (lambda a: (lambda t: t.astype(jnp.bfloat16) if jnp.issubdtype(t.dtype, jnp.floating) else t)(jnp.asarray(a)))
    def _A_setup():
        B, Sq, D = 8, 224, 512
        Hq, Hkv, Sk, Dh = 32, 32, 512, 128
        assert Hq % Hkv == 0, (Hq, Hkv)
        return {
            "x": _w((lambda *s: _rng.normal(s) * 0.8)(B, Sq, D)),
            "k_cache": _w((lambda *s: _rng.normal(s) * 0.8)(B, Hkv, Sk, Dh)),
            "v_cache": _w((lambda *s: _rng.normal(s) * 0.05)(B, Hkv, Sk, Dh)),
            "wq": _w((lambda *s: _rng.normal(s) * 0.8)(D, Hq * Dh) * (D ** -0.5)),
            "wo": _w((lambda *s: _rng.normal(s) * 0.05)(Hq * Dh, D) * ((Hq * Dh) ** -0.5)),
        }
    _A_in = _A_setup()

    def _B_setup():
        B, Sq, D = 8, 224, 512
        H, Sk, Dh = 32, 512, 128
        return {
            "x": _w((lambda *s: _rng.normal(s) * 0.8)(B, Sq, D)),
            "k_cache": _w((lambda *s: _rng.normal(s) * 0.8)(B, H, Sk, Dh)),
            "v_cache": _w((lambda *s: _rng.normal(s) * 0.05)(B, H, Sk, Dh)),
            "wq": _w((lambda *s: _rng.normal(s) * 0.8)(D, H * Dh) * (D ** -0.5)),
            "wo": _w((lambda *s: _rng.normal(s) * 0.05)(H * Dh, D) * ((H * Dh) ** -0.5)),
        }
    _B_in = _B_setup()

    return {
        "A_x": _A_in["x"],
        "A_k_cache": _A_in["k_cache"],
        "A_v_cache": _A_in["v_cache"],
        "A_wq": _A_in["wq"],
        "A_wo": _A_in["wo"],
        "B_x": _B_in["x"],
        "B_k_cache": _B_in["k_cache"],
        "B_v_cache": _B_in["v_cache"],
        "B_wq": _B_in["wq"],
        "B_wo": _B_in["wo"],
    }

def reference(A_x, A_k_cache, A_v_cache, A_wq, A_wo, B_x, B_k_cache, B_v_cache, B_wq, B_wo):
    def _A_ref(x, k_cache, v_cache, wq, wo):
        B, Sq, D = x.shape
        Hq, Dh = 32, 128
        Hkv = k_cache.shape[1]
        rep = Hq // Hkv
        q = (lambda x, *d: x.transpose(*d))((x @ wq).reshape(B, Sq, Hq, Dh), 0, 2, 1, 3)
        k = jnp.repeat(k_cache, rep, axis=1)
        v = jnp.repeat(v_cache, rep, axis=1)
        scores = jnp.einsum("bhqd,bhkd->bhqk", q, k) * (Dh ** -0.5)
        p = _softmax(scores, axis=-1)
        o = jnp.einsum("bhqk,bhkd->bhqd", p, v)
        return (lambda x, *d: x.transpose(*d))(o, 0, 2, 1, 3).reshape(B, Sq, Hq * Dh) @ wo

    def _B_ref(x, k_cache, v_cache, wq, wo):
        B, Sq, D = x.shape
        H, Dh = 32, 128
        q = (lambda x, *d: x.transpose(*d))((x @ wq).reshape(B, Sq, H, Dh), 0, 2, 1, 3)
        scores = jnp.einsum("bhqd,bhkd->bhqk", q, k_cache) * (Dh ** -0.5)
        p = _softmax(scores, axis=-1)
        o = jnp.einsum("bhqk,bhkd->bhqd", p, v_cache)
        return (lambda x, *d: x.transpose(*d))(o, 0, 2, 1, 3).reshape(B, Sq, H * Dh) @ wo

    a = _A_ref(A_x, A_k_cache, A_v_cache, A_wq, A_wo)
    b = _B_ref(B_x, B_k_cache, B_v_cache, B_wq, B_wo)
    return jnp.concatenate([a, b], axis=-1)
```

```python
import contextlib, functools, math, itertools
import jax, jax.numpy as jnp
from jax import lax
import jax.experimental.pallas as pl
import jax.experimental.pallas.tpu as pltpu

f32, bf16, u32 = jnp.float32, jnp.bfloat16, jnp.uint32
B, Sq, D, H, Sk, Dh = 8, 224, 512, 32, 512, 128

S_LHS = [{(0,0):1,(1,1):1}, {(1,0):1,(1,1):1}, {(0,0):1}, {(1,1):1}, {(0,0):1,(0,1):1}, {(1,0):1,(0,0):-1}, {(0,1):1,(1,1):-1}]
S_RHS = [{(0,0):1,(1,1):1}, {(0,0):1}, {(0,1):1,(1,1):-1}, {(1,0):1,(0,0):-1}, {(1,1):1}, {(0,0):1,(0,1):1}, {(1,0):1,(1,1):1}]
S_OUT = {(1,0):{1:1,3:1}, (0,1):{2:1,4:1}, (0,0):{0:1,3:1,4:-1,6:1}, (1,1):{0:1,1:-1,2:1,5:1}}
INNER4 = {0: (1,3,0,6,2,4,5), 3: (6,0,1,3,4,2,5), 2: (1,3,0,6,4,2,5), 1: (2,4,5,1,3,0,6)}
INNER2 = {0: (1,3,0,6,4,2,5), 1: (6,0,4,2,5,1,3)}

def lin(terms):
    terms = sorted(terms, key=lambda t: -t[0])
    s, acc = terms[0]
    assert s > 0
    for s, v in terms[1:]:
        acc = acc + v if s > 0 else acc - v
    return acc
def slin(terms):
    if max(s for s, _ in terms) > 0: return 1, lin(terms)
    return -1, lin([(-s, v) for s, v in terms])

def combiner(tab, load):
    load = functools.cache(load)
    @functools.cache
    def mid(p1, r0, c0):
        return lin([(s, load(2*r1+r0, 2*c1+c0)) for (r1, c1), s in tab[p1].items()])
    return lambda p1, p0: lin([(s, mid(p1, *rc)) for rc, s in tab[p0].items()])
def blocks_of(tab, p1, p0):
    return {(2*r1+r0, 2*c1+c0) for (r1,c1) in tab[p1] for (r0,c0) in tab[p0]}

class Gather:
    def __init__(self, park):
        self.park, self.held, self.cnt = park, {ij: [] for ij in S_OUT}, {ij: 0 for ij in S_OUT}
    def push(self, wave):
        outs, open_ = [], []
        for ij, t in S_OUT.items():
            new = [(t[p], p) for p in wave if p in t]
            if not new: continue
            self.cnt[ij] += len(new)
            if self.cnt[ij] == len(t):
                outs.append((ij, lin([(s, wave[p]) for s, p in new] + [(s, get()) for s, get in self.held[ij]])))
            else:
                open_.append((ij, new))
        raw = sorted({p for _, new in open_ for _, p in new})
        if len(raw) < len(open_):
            got = {p: self.park(wave[p]) for p in raw}
            for ij, new in open_: self.held[ij] += [(s, got[p]) for s, p in new]
        else:
            for ij, new in open_:
                s, v = slin([(s, wave[p]) for s, p in new])
                self.held[ij].append((s, self.park(v)))
        return outs

class Gather2:
    def __init__(self, park):
        self.inner = [Gather(park) for _ in range(7)]
        self.outer = {ij: Gather(park) for ij in S_OUT}
    def push(self, got):
        by, mids, outs = {}, {}, []
        for (p1, p0), v in got.items(): by.setdefault(p1, {})[p0] = v
        for p1, w in by.items():
            for ij0, v in self.inner[p1].push(w): mids.setdefault(ij0, {})[p1] = v
        for ij0, w in mids.items():
            for ij1, v in self.outer[ij0].push(w):
                outs.append(((2*ij1[0]+ij0[0], 2*ij1[1]+ij0[1]), v))
        return outs

flip = lambda i: i ^ 3
CHUNKS = [(e, i1, j1) for (i1, j1) in S_OUT for e in range(2)]
QG = {0: [(e, p1) for pp in ((1,3),(2,4),(0,6),(5,)) for e in range(2) for p1 in pp],
      1: [(0,1),(0,3),(0,2),(0,4),(0,0),(1,1),(1,3),(1,2),(1,4),(0,6),(1,0),(1,6),(0,5),(1,5)]}
def expand(tokens, prefix=False, qfirst=0, oorder=(2,3,0,1,5,4,6), inner2=INNER2):
    qg, og = list(QG[qfirst]), list(oorder)
    qcur, ocur, steps, ready, done, seen, nk, npv = [], [], [], [], set(), {}, 0, 0
    for ch in tokens:
        if ch == "K":
            assert nk < len(ready)
            steps.append(("K", ready[nk])); nk += 1
        elif ch == "P":
            assert npv < nk
            steps.append(("P", ready[npv])); done.add(ready[npv]); npv += 1
        elif ch in "xw":
            steps.append((ch, None))
        else:
            w, pos = [], 0
            assert ch == "O" or qcur or qg
            while ch == "Q" and pos < 4 and (qcur or qg):
                if not qcur:
                    e, p1 = qg.pop(0)
                    qcur = [(e, p1, p0) for p0 in INNER4[pos]]
                e, p1, p0 = qcur.pop(0)
                w.append(("Q", e, p1, p0)); seen.setdefault(e, set()).add((p1, p0)); pos += 1
            while pos < 4:
                if not ocur:
                    assert og
                    p1 = og.pop(0)
                    ocur = [(p1, p0) for p0 in inner2[pos // 2]]
                p1, p0 = ocur.pop(0)
                assert all((e, flip(i), k) in done for e in range(2) for i, k in blocks_of(S_LHS, p1, p0))
                w.append(("O", 0, p1, p0)); pos += 2
            for e, sn in seen.items():
                for ij1, t1 in S_OUT.items():
                    for ij0, t0 in S_OUT.items():
                        u = (e, 2*ij1[0]+ij0[0], 2*ij1[1]+ij0[1])
                        if u not in ready and all((a, b) in sn for a in t1 for b in t0): ready.append(u)
            ready[nk:] = sorted(ready[nk:], key=lambda u: CHUNKS.index((u[0], u[1] // 2, u[2] // 2)))
            steps.append(("W", w))
    assert prefix or (not (qg or og or qcur or ocur) and npv == 32)
    return steps

PB = "w" + "QQQ" + ("KQP"*2 + "KQPQ")*3 + "KOPQ" + "KQP" + "KOPQ" + "KQP" + "KOPQ" + "KQP"*5 + "KOP"*13 + "O"*8
PA = "w" + "Q"*8 + "wQ" + "KQP"*3 + "KQwP" + "KQP"*4 + "KQP"*3 + "KQwPx" + "KOPx"*3 + "KQxxxxwPx" + "KOPx"*3 + "KQxxxxwPx" + "KQPx"*2 + "KOP"*5 + "KOxxxxwP" + "KOP"*4 + "O"*8 + "xxxx"

def build(pa=PA, pb=PB, t1=3, flags=None, verbose=0, pk=1, park_s=4, nobc=1, nosc=1, of32=0, only=None, scopes=0, dpos=(1,4,6,0), inner2=INNER2, oorder=(2,3,0,1,5,4,6)):
    c = (Dh ** -0.5) * math.log2(math.e)
    T, W = 16, 1024
    def ld(ref, *idx):
        return pltpu.bitcast(ref.bitcast(u32)[idx], bf16) if pk else ref[idx]
    plans = [expand(pa, qfirst=1, inner2=inner2, oorder=oorder), expand(pb, inner2=inner2, oorder=oorder)]
    if verbose:
        for n, steps in enumerate(plans):
            if only is None or only == n:
                print(" ".join(("[" + " ".join(f"{x[0]}{x[1]}.{x[2]}{x[3]}" for x in a) + "]") if k == "W" else f"{k}{a[0]}.{a[1]}{a[2]}" for k, a in steps if k not in "xw"))
    def uses(k, a):
        if k == "K": return [("k", (a[0], a[1] // 2, a[2] // 2))]
        if k == "P": return [("v", (a[0], a[1] // 2, a[2] // 2))]
        if k == "W": return [("wq", x[1]) if x[0] == "Q" else ("wo", 0) for x in a]
        if k == "x": return [("x", 0)]
    def stream(steps):
        groups, seen = [], []
        for k, a in steps:
            if k == "w": groups.append([]); continue
            for it in uses(k, a):
                if it not in seen: seen.append(it); groups[-1].append(it)
        return groups
    streams = [stream(plans[0]), [[("wq", None), ("k", None), ("v", None), ("wo", 0)]]]
    NW = ahead = len(streams[0])

    def kernel(ax, ak, av, awq, awo, bx, bk, bv, bwq, bwo, out,
               xs, xc, kb, vb, wqs, wos, qs, ss, ps, qt, ot, acc, ob, sem, osem):
        X, K, V, WQ, WO = (ax, bx), (ak, bk), (av, bv), (awq, bwq), (awo, bwo)
        def x_copy(g, sm):
            return pltpu.make_async_copy(X[g // 2].at[pl.ds(4*(g % 2), 4)], xs.at[g], sm)
        def transfer(op, r, t, items, grp):
            hp, z = (t >> 1) & 3, t & 1
            sm = sem.at[z, grp]
            for kind, part in items:
                if kind == "x":
                    for g in range(1, 4): pl.when(t == g - 1)(lambda g=g: op(x_copy(g, sm)))
                elif kind == "wo":
                    pl.when(z == 0)(lambda: op(pltpu.make_async_copy(WO[r].at[pl.ds(pl.multiple_of(hp*W, W), W), :], wos.at[hp & 1], sm)))
                elif kind == "wq":
                    o, n = (0, W) if part is None else (512*part, 512)
                    pl.when(z == 0)(lambda: op(pltpu.make_async_copy(WQ[r].at[:, pl.ds(pl.multiple_of(hp*W + o, 512), n)], wqs.at[hp & 1, :, pl.ds(o, n)], sm)))
                else:
                    src, dst = (K, kb) if kind == "k" else (V, vb)
                    b0, nb, h0, nh = (0, 4, 0, 8) if part is None else (2*part[1], 2, 4*part[0] + 2*part[2], 2)
                    op(pltpu.make_async_copy(src[r].at[pl.ds(4*z + b0, nb), pl.ds(8*hp + h0, nh)], dst.at[z, pl.ds(b0, nb), pl.ds(h0, nh)], sm))
        start, wait = (lambda cp: cp.start()), (lambda cp: cp.wait())
        def x_combos(g, r0, part=range(7)):
            rows = pl.ds(r0 if isinstance(r0, int) else pl.multiple_of(r0, 16), 16)
            pair = functools.cache(lambda i, k1: xs[g, i, rows, k1*256:(k1+1)*256].astype(f32) * c)
            cx = combiner(S_LHS, lambda i, k: pair(i, k // 2)[:, (k % 2)*128:(k % 2 + 1)*128])
            for p1 in part:
                for p0 in range(7):
                    xc[g, 7*p1 + p0, rows, :] = cx(p1, p0).astype(bf16)

        x_copy(0, osem).start()
        for grp in range(ahead):
            @pl.loop(16*grp // ahead, 16*(grp + 1) // ahead)
            def _(n):
                acc[n >> 2, n & 3] = jnp.zeros(acc.shape[2:], f32)
            transfer(start, 0, 0, streams[0][grp], grp)
        with (jax.named_scope(f"wait_x") if scopes else contextlib.nullcontext()):
            x_copy(0, osem).wait()
        @pl.loop(0, Sq // 16)
        def _(i):
            x_combos(0, i*16)

        def body(mode, t):
            steps, groups = plans[mode], streams[mode]
            r, hp, z = t >> 3, (t >> 1) & 3, t & 1
            g, wz = 2*r + z, hp & 1
            o0, o1 = t >> 4, t >> 5
            nx = sum(k == "x" for k, _ in steps)
            work = [(sl, p1) for sl in range(14) for p1 in range(7)]
            todo_x = [work[len(work)*a // nx:len(work)*(a + 1) // nx] for a in range(nx)]
            def parker(ref):
                cnt = itertools.count()
                def park(v):
                    n = next(cnt)
                    assert n < ref.shape[1]
                    ref[o0, n] = v
                    return lambda: ref[o0, n]
                return park
            qpark = parker(qt)
            qgath, ogath = [Gather2(qpark) for _ in range(2)], Gather2(parker(ot))
            def wcomb(load):
                pair = functools.cache(lambda k, j1: load(k, j1).astype(f32))
                return combiner(S_RHS, lambda k, j: pair(k, j // 2)[:, (j % 2)*128:(j % 2 + 1)*128])
            def wave(w):
                wq = [wcomb(lambda k, j1, e=e: wqs[wz, k*128:(k+1)*128, e*512 + j1*256:e*512 + (j1+1)*256]) for e in range(2)]
                wo = [wcomb(lambda k, j1, e=e: wos[wz, e*512 + k*128:e*512 + (k+1)*128, j1*256:(j1+1)*256]) for e in range(2)]
                co = [combiner(S_LHS, lambda i, k, e=e: ss[o0, e, flip(i), k]) for e in range(2)]
                gq, go = {}, {}
                for kind, e, p1, p0 in w:
                    if kind == "Q":
                        gq.setdefault(e, {})[p1, p0] = jnp.dot(ld(xc, g, 7*p1+p0), wq[e](p1, p0).astype(bf16), preferred_element_type=f32)
                    else:
                        m = [jnp.dot(co[d](p1, p0).astype(f32 if of32 else bf16), wo[d](p1, p0).astype(bf16), preferred_element_type=f32) for d in range(2)]
                        go[p1, p0] = m[0] + m[1]
                for e, got in gq.items():
                    for (i, j), v in qgath[e].push(got): qs[o0, e, i, j] = v.astype(bf16)
                for (i, j), v in ogath.push(go):
                    i = flip(i)
                    y = acc[g, i, j] + v
                    acc[g, i, j] = y
                    if mode:
                        ob[g, j, i] = y.astype(bf16)
                        pl.when(hp == 3)(lambda: pltpu.make_async_copy(ob.at[g, j, i], out.at[4*z + i, :, pl.ds(pl.multiple_of(r*D + j*128, 128), 128)], osem).start())
            keep = {}
            def qk(e, i, j):
                s = lax.dot_general(ld(qs, o0, e, i, j), ld(kb, z, i, 4*e + j), (((1,), (1,)), ((), ())), preferred_element_type=f32)
                m = jnp.max(s, axis=-1, keepdims=True)
                sk = [s[:, k*128:(k+1)*128] for k in range(4)]
                for k in range(park_s):
                    ss[o0, 2, j, k] = sk[k]
                    sk[k] = ss[o0, 2, j, k]
                pe = [jnp.exp2(sk[k] - m) for k in range(4)]
                for k in range(4): ps[o0, j, k] = pe[k].astype(bf16)
                l = jnp.sum((pe[0] + pe[1]) + (pe[2] + pe[3]), axis=-1, keepdims=True)
                keep[e, i, j] = pltpu.reciprocal(l, approx=True)
            def pv(e, i, j, base):
                p = jnp.concatenate([ld(ps, o0, j, k) for k in range(4)], axis=-1)
                ss[base, e, i, j] = jnp.dot(p, ld(vb, z, i, 4*e + j), preferred_element_type=f32) * keep.pop((e, i, j))
            lastk = max(n for n, (k, a) in enumerate(steps) if k == "K")
            nwait = itertools.count()
            for n, (k, a) in enumerate(steps):
                if k == "W": wave(a)
                elif k == "K": qk(*a)
                elif k == "P": pv(*a, o1 if n < lastk else o0)
                elif k == "w":
                    a = next(nwait)
                    with (jax.named_scope(f"wait{mode}_{a}") if scopes else contextlib.nullcontext()):
                        transfer(wait, 0, t, groups[a], a)
                    if mode == 0:
                        transfer(start, 0, t + 1, groups[a], jnp.where(t + 1 < t1, a, 0))
                else:
                    pc = todo_x.pop(0)
                    for sl in sorted({sl for sl, _ in pc}):
                        x_combos(jnp.minimum(t + 1, 3), sl*16, [p1 for s2, p1 in pc if s2 == sl])
                if mode and n in dpos:
                    for rr in range(2):
                        pl.when(((t + 1) >> 3) == rr)(lambda: transfer(start, rr, t + 1, [it for it, p in zip(groups[0], dpos) if p == n], 0))
        if only in (None, 0): pl.loop(0, t1)(functools.partial(body, 0))
        if only in (None, 1): pl.loop(t1, T)(functools.partial(body, 1))
        pltpu.make_async_copy(ob, ob, osem).wait()

    def fn(*args):
        return pl.pallas_call(
            kernel,
            in_specs=[pl.BlockSpec(memory_space=pl.ANY)]*10,
            out_specs=pl.BlockSpec(memory_space=pl.ANY),
            out_shape=jax.ShapeDtypeStruct((B, Sq, 2*D), bf16),
            scratch_shapes=[
                pltpu.VMEM((4, 4, Sq, D), bf16),
                pltpu.VMEM((4, 49, Sq, 128), bf16),
                pltpu.VMEM((2, 4, 8, Sk, Dh), bf16),
                pltpu.VMEM((2, 4, 8, Sk, Dh), bf16),
                pltpu.VMEM((2, D, W), bf16),
                pltpu.VMEM((2, W, D), bf16),
                pltpu.VMEM((1, 2, 4, 4, Sq, Dh), bf16),
                pltpu.VMEM((1, 3, 4, 4, Sq, 128), f32),
                pltpu.VMEM((1, 4, 4, Sq, 128), bf16),
                pltpu.VMEM((1, 80, Sq, Dh), f32),
                pltpu.VMEM((1, 60, Sq, Dh), f32),
                pltpu.VMEM((4, 4, 4, Sq, 128), f32),
                pltpu.VMEM((4, 4, 4, Sq, 128), bf16),
                pltpu.SemaphoreType.DMA((2, NW)),
                pltpu.SemaphoreType.DMA(()),
            ],
            compiler_params=pltpu.CompilerParams(vmem_limit_bytes=100*2**20, flags=flags, disable_bounds_checks=bool(nobc), disable_semaphore_checks=bool(nosc)),
        )(*args)
    return fn


@jax.jit
def pallas_concat_heads__gqa_block_cached__mha_block_cached__near_ridge_kernel(
    A_x, A_k_cache, A_v_cache, A_wq, A_wo, B_x, B_k_cache, B_v_cache, B_wq, B_wo):
    return build()(A_x, A_k_cache, A_v_cache, A_wq, A_wo, B_x, B_k_cache, B_v_cache, B_wq, B_wo)
```

```python
import functools
import itertools
import math

import jax
import jax.experimental.pallas as pl
import jax.experimental.pallas.tpu as pltpu
import jax.numpy as jnp
from jax import lax

B, SQ, D, H, SK, DH = 8, 224, 512, 32, 512, 128
TB, TH = 4, 8
NTILE = 2 * (H // TH) * (B // TB)
HALF = SQ // 2
NMXU = 4
LOGIT_SCALE = DH ** -0.5 * math.log2(math.e)

_reciprocal = pltpu.reciprocal if hasattr(pltpu, "reciprocal") else pl.reciprocal


def _scheme(table):
    def parse(t):
        return {(int(t[n + 1]), int(t[n + 2])): int(t[n] + "1") for n in range(0, len(t), 3)}

    lhs, rhs, out = zip(*[map(parse, line.split()) for line in table.strip().splitlines()])
    tensor = {}
    for a, b, c in zip(lhs, rhs, out):
        for key, signs in zip(itertools.product(a, b, c), itertools.product(a.values(), b.values(), c.values())):
            tensor[key] = tensor.get(key, 0) + math.prod(signs)
    blocks = dict.fromkeys(ij for o in out for ij in o)
    depth = 1 + max(k for a in lhs for _, k in a)
    assert {key: v for key, v in tensor.items() if v} == {
        ((i, k), (k, j), (i, j)): 1 for i, j in blocks for k in range(depth)
    }
    return lhs, rhs, {ij: {p: o[ij] for p, o in enumerate(out) if ij in o} for ij in blocks}


STRASSEN = _scheme("""
+00+11  +00+11  +00+11
+10+11  +00     +10-11
+00     +01-11  +01+11
+11     +10-00  +10+00
+00+01  +11     +01-00
+10-00  +00+01  +11
+01-11  +10+11  +00
""")

HOPCROFT_KERR = _scheme("""
+30              +01-11-21     +01+31-11
+20              +00-30        +20-10
+30+32           +11+20-10-21  +01-31
+22              +21+30-20-31  +00-20
+11-30           +00-11-20     +01-11-30
+11              +10+20-00     +10-30-00
+30+32-11-01     +10-11-20     +01-30-31
+11+01           +10-20        +00+01-30-31
+13-20           +01-30        -10-21
+13              +31-01        +11-21
+03-22           +21+30-31     +00-20-21
+03              +31-21        +00+01-20-21
+10+13+00        +01           +10+11
+00-11           +00-20        +00+01-10-11
+10+12+20        +00-01        +10
+12-00           +00-01-20     +01-10-11
+30-12           +00+21-01-20  +01-11
+11+00+01+02+22  +20           +00
+12+30+32+02+03  +21           +01
+11+30+31+32+21  +10-11        +30
+21              +10-30        +20-30
+11+30+31+33+01  +11           +30+31
+33-21           +11-30        -30-21
+33              +31-11        +31-21
+13+33+22+23     +31-30        +21
+03+20+21+23     +30           +20+21
""")

INNER_ORDER = ((1, 3, 0, 6, 2, 4, 5), (2, 4, 5, 1, 3, 0, 6), (1, 3, 0, 6, 4, 2, 5), (6, 0, 1, 3, 4, 2, 5))
NEVER = 99


class _Recombiner:
    def __init__(self, out, slots, first=None):
        self.out, self.slots = out, slots
        self.missing = {ij: len(t) for ij, t in out.items()}
        self.held = {ij: [(1, first(ij))] if first else [] for ij in out}

    def push(self, new, stores, fold):
        def park(terms):
            sign = max(s for s, _ in terms)
            key = ("slot", next(self.slots))
            stores.append((key, [(s * sign, v) for s, v in terms]))
            return sign, key

        finished, waiting = {}, {}
        for ij, signs in self.out.items():
            terms = [(signs[p], v) for p, v in new.items() if p in signs]
            self.missing[ij] -= len(terms)
            if terms and not self.missing[ij]:
                finished[ij] = tuple(terms + self.held[ij])
            elif terms and len(self.held[ij]) >= fold:
                self.held[ij] = [park(terms + self.held[ij])]
            elif terms:
                waiting[ij] = terms
        raw = dict.fromkeys(v for terms in waiting.values() for _, v in terms)
        if len(raw) < len(waiting):
            raw = {v: park([(1, v)])[1] for v in raw}
            for ij, terms in waiting.items():
                self.held[ij] += [(s, raw[v]) for s, v in terms]
        else:
            for ij, terms in waiting.items():
                self.held[ij].append(park(terms))
        return finished


def _plan_waves(outer, groups, widths, folds, carry=False):
    slots = itertools.count()
    block = lambda hi, lo: (2 * hi[0] + lo[0], 2 * hi[1] + lo[1])
    inner = {g: _Recombiner(STRASSEN[2], slots) for g in groups}
    top = {
        (e, lo): _Recombiner(outer[2], slots, carry and (lambda hi, lo=lo: ("carry", block(hi, lo))))
        for e in dict.fromkeys(e for e, _ in groups)
        for lo in STRASSEN[2]
    }
    todo, current, waves = list(groups), [], []
    for width, fold in zip(widths, folds, strict=True):
        products, stores, low, mid = [], [], {}, {}
        for mxu in range(NMXU - width, NMXU):
            if not current:
                e, hi = todo.pop(0)
                current = [(e, hi, lo) for lo in INNER_ORDER[mxu]]
            e, hi, lo = current.pop(0)
            low.setdefault((e, hi), {})[lo] = ("product", len(products))
            products.append((e, hi, lo))
        for (e, hi), new in low.items():
            for lo, terms in inner[e, hi].push(new, stores, NEVER).items():
                mid.setdefault((e, lo), {})[hi] = ("sum", terms)
        for (e, lo), new in mid.items():
            for hi, terms in top[e, lo].push(new, stores, fold).items():
                stores.append((("result", (e,) + block(hi, lo)), terms))
        waves.append((products, stores))
    assert not todo and not current and not any(n for r in top.values() for n in r.missing.values())
    return waves, next(slots)


def _signed_sum(terms):
    (sign, total), *rest = sorted(terms, key=lambda t: -t[0])
    assert sign > 0
    for sign, v in rest:
        total = total + v if sign > 0 else total - v
    return total


def _operands(outer, inner, load):
    load = functools.cache(load)

    @functools.cache
    def mid(hi, r, c):
        return _signed_sum([(s, load(2 * rr + r, 2 * cc + c)) for (rr, cc), s in outer[hi].items()])

    def operand(hi, lo):
        return _signed_sum([(s, mid(hi, *rc)) for rc, s in inner[lo].items()]).astype(jnp.bfloat16)

    return operand


N_EARLY = 3
PLAN_FIRST = "wQsQQQQQQQQQQQwQsKQPcKQPQcKQPcwQsKQPcKQPcKQPcKQPcKQPcwQsKoPoKoPoKoPc"
PLAN_NEXT = "wwwwQttQtQQQtstQtsQQQQQQQKQPcKQPQcKQPcQKQPcKsQPcKQPcKQPcKQPcKQPocKoPsooKoP"
PLAN_REST = "wKsoPoKoPoKoPocKoPKoPccKoPwKsoPcKoPKooPcKoPoKoPoKoPooKoPowKsoPKoPKoPcKoPQoKoPoKoPooKoPoKocP"
PLAN_STEADY = (
    "wQttQtQssQKtPtKQtPcxKssQxPQQxcKocPKQPcKoQPxcQKxQPQcKoPoxcKoPQxcKQPxQxccQKoPoKoPxcKQPoxKQP"
    "cxQoKoQPcxcKoPxcrKoPoKQPxQrKoPoxrKooPocKoPKoPorKoPooKorPKoPoKQPoKoPQKoPoKoPoKoPooKoPoKoPx"
)
O_FOLD = "2955353594545551411452519432329214911244959999"

UNITS = [
    (b0 + b, h0 + 4 * e + h)
    for b0, h0 in ((2, 0), (0, 2), (0, 0), (2, 2))
    for e in range(2)
    for b in (1, 0)
    for h in range(2)
]
O_WAVES, O_SLOTS = _plan_waves(
    HOPCROFT_KERR, [(0, hi) for hi in range(26)], [2] + [4] * 45, map(int, O_FOLD), carry=True
)
(Q_EARLY, _n0), (Q_STEADY, _n1) = (
    _plan_waves(STRASSEN, groups, [4] * 24 + [2], [NEVER] * 25)
    for groups in (
        [(e, hi) for e in range(2) for hi in (1, 3, 2, 4, 0, 6, 5)],
        [(e, hi) for his in ((1, 3), (2, 4), (0, 6), (5,)) for e in range(2) for hi in his],
    )
)
Q_SLOTS = max(_n0, _n1)
N_IN_TILE = PLAN_STEADY.count("o")


def _steps(plan, q_waves):
    def reads(n):
        return {
            (b, 2 * j + h)
            for _, hi, lo in O_WAVES[n][0]
            for b, j in HOPCROFT_KERR[0][hi]
            for _, h in STRASSEN[0][lo]
        }

    count, steps, have_q, have_o = dict.fromkeys("KPQotwsxcr", 0), [], set(), set()
    for kind in plan:
        n = count[kind]
        count[kind] += 1
        if kind == "t":
            n += N_IN_TILE
            assert not reads(n) & have_o and not count["o"] and count["s"] < 4
        if kind == "Q":
            have_q |= {(k[1][1], 4 * k[1][0] + k[1][2]) for k, _ in q_waves[n][1] if k[0] == "result"}
        if kind == "K":
            assert UNITS[n] in have_q and n == count["P"]
        if kind == "P":
            assert count["K"] == count["P"]
            have_o.add(UNITS[n])
        if kind == "o":
            assert reads(n) <= have_o
        if kind == "s":
            assert count["w"] > n or count["w"] == plan.count("w")
        steps.append((kind, n))
    assert (count["P"], count["Q"], count["o"]) == (len(UNITS), len(q_waves), N_IN_TILE)
    assert count["t"] in (0, len(O_WAVES) - N_IN_TILE) and count["c"] == 16
    assert (count["x"], count["r"]) in ((0, 0), (17, 5))
    return steps


def _fetch_groups(steps, q_waves):
    groups, seen = [], set()
    for kind, n in steps:
        needs = []
        if kind == "w":
            groups.append([])
        elif kind in "KP":
            needs = [("k" if kind == "K" else "v", UNITS[n][0], 1, UNITS[n][1], 1)]
        elif kind == "Q":
            needs = [("wq", 0, D, 4 * DH * e, 4 * DH) for e, _, _ in q_waves[n][0]]
        elif kind == "c" and n < 8:
            needs = [("wq", 0, D, 4 * DH * (n // 4), 4 * DH)]
        elif kind in "oc":
            needs = [("wo", 0, 0, 0, 0)]
        for item in needs:
            if item not in seen:
                seen.add(item)
                groups[-1].append(item)
    for group in groups:
        for a, b in ((3, 1), (1, 3)):
            merged = []
            for it in sorted(group, key=lambda it: (it[0], it[b:b + 2], it[a])):
                last = merged[-1] if merged else None
                if last and (last[0], last[b:b + 2], last[a] + last[a + 1]) == (it[0], it[b:b + 2], it[a]):
                    merged[-1] = last[:a + 1] + (last[a + 1] + it[a + 1],) + last[a + 2:]
                else:
                    merged.append(it)
            group[:] = merged
    return groups


EARLY_STEPS = _steps(PLAN_FIRST + PLAN_REST, Q_EARLY)
NEXT_STEPS = _steps(PLAN_NEXT + PLAN_REST, Q_EARLY)[:len(PLAN_NEXT)]
assert sorted(PLAN_FIRST) == sorted(PLAN_NEXT.replace("t", ""))
STEADY_STEPS = _steps(PLAN_STEADY, Q_STEADY)
PIECEWISE = _fetch_groups(EARLY_STEPS, Q_EARLY)
WHOLE = [("wq", 0, D, 0, TH * DH), ("k", 0, TB, 0, TH), ("v", 0, TB, 0, TH), ("wo", 0, 0, 0, 0)]


W_HIGH_SPREAD = 2.25
W_LOW_SPREAD = 3.0
Q_SPREAD = 3.5
OUT_SPREAD = 2.75


def _comparable(large, small, spread):
    return (large <= spread * small) & (small > 1e-30) & (large < 1e30)


def _packed(ref, *idx):
    return pltpu.bitcast(ref.bitcast(jnp.uint32)[idx], jnp.bfloat16)


def _kernel(ax, ak, av, awq, awo, bx, bk, bv, bwq, bwo, out,
            x_raw, x_ops, k_buf, wq_buf, wo_buf, v_buf, q_buf, so_buf, p_buf, q_part, o_part, o_size, carry,
            out_buf, q_size, in_sem, x_sem, out_sem):
    f32, bf16 = jnp.float32, jnp.bfloat16
    x_hbm, wq_hbm, wo_hbm = (ax, bx), (awq, bwq), (awo, bwo)
    kv = {"k": ((ak, bk), k_buf), "v": ((av, bv), v_buf)}
    start, wait = (lambda copy: copy.start()), (lambda copy: copy.wait())
    lanes = lambda v, n: v[:, 128 * n:128 * (n + 1)]

    def x_copy(branch, bg):
        g = 2 * branch + bg
        return pltpu.make_async_copy(x_hbm[branch].at[pl.ds(TB * bg, TB)], x_raw.at[g], x_sem.at[g])

    def transfer(op, branch, t, items, nsem):
        hg, bg = (t >> 1) & 3, t & 1
        sem = in_sem.at[nsem]
        for name, r0, nr, c0, nc in items:
            if name == "wq":

                @pl.when(bg == 0)
                def _():
                    cols = pl.ds(pl.multiple_of(hg * TH * DH + c0, DH), nc)
                    op(pltpu.make_async_copy(wq_hbm[branch].at[:, cols], wq_buf.at[hg & 1, :, pl.ds(c0, nc)], sem))

            elif name == "wo":
                @pl.when(bg == 0)
                def _():
                    rows = pl.ds(pl.multiple_of(hg * TH * DH, DH), TH * DH)
                    for j in range(4):
                        cols = pl.ds(pl.multiple_of(((j + hg) & 3) * 128, 128), 128)
                        op(pltpu.make_async_copy(wo_hbm[branch].at[rows, cols], wo_buf.at[hg & 1, j], sem))

            else:
                src, dst = kv[name]
                op(pltpu.make_async_copy(
                    src[branch].at[pl.ds(TB * bg + r0, nr), pl.ds(TH * hg + c0, nc)],
                    dst.at[bg, pl.ds(r0, nr), pl.ds(c0, nc)], sem))

    def send(t, b0, nb):
        branch, bg = t >> 3, t & 1
        for j in range(4):
            cols = pl.ds(pl.multiple_of(D * branch + 128 * ((j + 3) % 4), 128), 128)
            pltpu.make_async_copy(
                out_buf.at[2 * branch + bg, j, pl.ds(b0, nb)], out.at[pl.ds(TB * bg + b0, nb), :, cols],
                out_sem.at[branch],
            ).start()

    def sent(branch):
        filled = out.at[:, :, pl.ds(D * branch, D)]
        pltpu.make_async_copy(filled, filled, out_sem.at[branch]).wait()

    def check_weights(n, t, zero):
        slot, bg = (t >> 1) & 1, t & 1
        if n < 8:
            rows = pl.ds(pl.multiple_of(256 * bg + 128 * (n % 2), 128), 128)
            pair = wq_buf[slot, rows, pl.ds(256 * (n // 2), 256)].astype(f32)
            blocks = [lanes(pair, 0), lanes(pair, 1)]
        else:
            rows = pl.ds(pl.multiple_of(256 * bg + 64 * (n % 8 // 2), 64), 64)
            blocks = [_packed(wo_buf, slot, 2 * (n % 2) + j, rows).astype(f32) for j in range(2)]
        state = so_buf.at[zero, TB + 1, 2 * (t >> 3) + n // 8]
        low, high, mean = (state[pl.ds(8 * i, 8)] for i in range(3))
        squares = [v * v for v in blocks]
        for square in squares:
            down = jnp.broadcast_to(jnp.sum(square, axis=0, keepdims=True), (8, 128))
            low, high = jnp.minimum(low, down), jnp.maximum(high, down)
            mean = jnp.maximum(mean, jnp.sum(down, axis=1, keepdims=True) * (1 / 128))
        both = squares[0] + squares[1]
        across = [jnp.sum(both[r:r + 8], axis=1, keepdims=True) for r in range(0, 128, 8)]
        high = jnp.maximum(high, 0.5 * functools.reduce(jnp.maximum, across))
        for i, v in enumerate((low, high, mean)):
            state[pl.ds(8 * i, 8)] = v

    def check_x(slab, zero):
        rows = pl.ds(pl.multiple_of(16 * (slab >> 2), 16), 16)
        x = [x_raw[slab & 3, b, rows].astype(f32) for b in range(TB)]
        mixed = jnp.sum(functools.reduce(jnp.add, [v * v for v in x]), axis=1, keepdims=True) * (1 / TB)
        high = (zero, TB + 1, slab & 2, pl.ds(32, 16))
        so_buf[high] = jnp.maximum(so_buf[high], mixed)

    def scores(q, k):
        return lax.dot_general(q, k, (((1,), (1,)), ((), ())), preferred_element_type=f32)

    def plain(i):
        branch, b = i >> 3, i & 7
        total = carry.at[0, 0, 0]
        total[...] = jnp.zeros(total.shape, f32)

        @pl.loop(0, H)
        def _(h):
            head = pl.ds(pl.multiple_of(DH * h, DH), DH)

            def copies(r):
                pairs = [
                    (kv["k"][0][r].at[b, h], k_buf.at[0, 0, 0]),
                    (kv["v"][0][r].at[b, h], v_buf.at[0, 0, 0]),
                    (wq_hbm[r].at[:, head], wq_buf.at[0, :, pl.ds(0, DH)]),
                    (wo_hbm[r].at[head, :], wq_buf.at[1, pl.ds(0, DH), pl.ds(0, D)]),
                ]
                return [pltpu.make_async_copy(src, dst, x_sem.at[n]) for n, (src, dst) in enumerate(pairs)]

            for r in range(2):

                @pl.when(branch == r)
                def _():
                    for op in (start, wait):
                        for copy in copies(r):
                            op(copy)

            @pl.loop(0, 2)
            def _(half):
                rows = pl.ds(pl.multiple_of(HALF * half, 16), HALF)
                q = jnp.dot(x_raw[i >> 2, i & 3, rows], wq_buf[0, :, pl.ds(0, DH)], preferred_element_type=f32)
                s = scores((q * LOGIT_SCALE).astype(bf16), k_buf[0, 0, 0])
                p = jnp.exp2(s - jnp.max(s, axis=-1, keepdims=True))
                o = jnp.dot(p.astype(bf16), v_buf[0, 0, 0], preferred_element_type=f32)
                o = (o / jnp.sum(p, axis=-1, keepdims=True)).astype(bf16)
                y = jnp.dot(o, wq_buf[1, pl.ds(0, DH), pl.ds(0, D)], preferred_element_type=f32)
                for j in range(4):
                    total[j, rows] += lanes(y, j)

        for j in range(4):
            out_buf[0, j, 0] = total[j].astype(bf16)
            cols = pl.ds(pl.multiple_of(D * branch + 128 * j, 128), 128)
            copy = pltpu.make_async_copy(out_buf.at[0, j, 0], out.at[b, :, cols], out_sem.at[0])
            copy.start()
            copy.wait()

    def x_slab(src, dst, row, products=range(49)):
        pair = functools.cache(lambda b, k: src[b, pl.ds(row, 16), pl.ds(256 * k, 256)].astype(f32))
        operand = _operands(STRASSEN[0], STRASSEN[0], lambda b, k: lanes(pair(b, k // 2), k % 2))
        for n in products:
            dst[n, pl.ds(row, 16)] = operand(n // 7, n % 7)

    def x_operands(g):
        x_copy(0, g).wait()

        @pl.loop(0, 2)
        def _(i):
            rows = pl.ds(pl.multiple_of(HALF * i, 16), HALF)
            for row in range(0, HALF, 16):
                x_slab(x_raw.at[g, :, rows], x_ops.at[g, :, rows], row)

    def run_wave(wave, lhs, rhs, part, zero, emit, load_carry=None):
        products, stores = wave
        done = []
        for e, hi, lo in products:
            a, b = lhs(hi, lo), rhs[e](hi, lo)
            cut = a.shape[0] // 32 * 16
            pieces = [a] if len(products) == NMXU else [a[:cut], a[cut:]]
            done.append(jnp.concatenate([jnp.dot(v, b, preferred_element_type=f32) for v in pieces]))

        @functools.cache
        def value(kind, arg):
            if kind == "sum":
                return _signed_sum([(s, value(*v)) for s, v in arg])
            if kind == "product":
                return done[arg]
            return part[zero, arg] if kind == "slot" else load_carry(*arg)

        for (kind, arg), terms in stores:
            total = value("sum", tuple(terms))
            if kind == "slot":
                part[zero, arg] = total
            else:
                emit(*arg, total)

    def q_wave(wave, t, zero):
        def weights(e):
            pair = functools.cache(
                lambda k, j: wq_buf[(t >> 1) & 1, pl.ds(128 * k, 128), pl.ds(512 * e + 256 * j, 256)].astype(f32)
            )
            return _operands(STRASSEN[1], STRASSEN[1], lambda k, j: lanes(pair(k, j // 2), j % 2))

        def emit(e, b, h, q):
            q_buf[zero, b, 4 * e + h] = (q * LOGIT_SCALE).astype(bf16)
            squares = [q[r:r + 8] * q[r:r + 8] for r in range(0, 128, 8)]
            size = jnp.sum(functools.reduce(jnp.add, squares), axis=0, keepdims=True)
            q_size[t >> 3] = jnp.minimum(q_size[t >> 3], size)

        g = 2 * (t >> 3) + (t & 1)
        lhs = lambda hi, lo: _packed(x_ops, g, 7 * hi + lo)
        run_wave(wave, lhs, [weights(0), weights(1)], q_part, zero, emit)

    def o_wave(n, t, zero, o_zero, may_be_last):
        hg, bg = (t >> 1) & 3, t & 1
        half = lambda i: pl.ds(HALF * (i % 2), HALF)
        acc = carry.at[bg, pl.ds(hg, 2)]

        def emit(_, i, j, y):
            acc[1, i // 2, j, half(i)] = y
            if may_be_last:
                out_buf[2 * (t >> 3) + bg, j, i // 2, half(i)] = y.astype(bf16)

        lhs = _operands(HOPCROFT_KERR[0], STRASSEN[0], lambda i, h: so_buf[o_zero, i // 2, h, half(i)])
        rhs = _operands(
            HOPCROFT_KERR[1], STRASSEN[1], lambda h, j: _packed(wo_buf, hg & 1, j, pl.ds(64 * h, 64)).astype(f32)
        )
        run_wave(O_WAVES[n], lhs, [rhs], o_part, zero, emit, lambda i, j: acc[0, i // 2, (j + 1) % 4, half(i)])

    def run(steady, steps, t):
        bg = t & 1
        zero, o_zero = t >> 4, t >> 5
        last = "P"
        for kind, n in steps:
            if kind in "KP":
                last, (b, h) = kind, UNITS[n]
            if kind == "K":
                s = scores(_packed(q_buf, zero, b, h), _packed(k_buf, bg, b, h))
                row_max = jnp.max(s, axis=-1, keepdims=True)
                for c in range(4):
                    so_buf[zero, TB, 4 * (n % 2) + c] = lanes(s, c)
                p = [jnp.exp2(so_buf[zero, TB, 4 * (n % 2) + c] - row_max) for c in range(4)]
                for c in range(4):
                    p_buf[zero, n % 2, c] = p[c].astype(bf16)
                total = jnp.sum((p[0] + p[1]) + (p[2] + p[3]), axis=-1, keepdims=True)
                norm = _reciprocal(total, approx=True)
                norm = norm * (2.0 - total * norm)
            elif kind == "P":
                p = jnp.concatenate([_packed(p_buf, zero, n % 2, c) for c in range(4)], axis=-1)
                o = jnp.dot(p, _packed(v_buf, bg, b, h), preferred_element_type=f32) * norm
                so_buf[o_zero, b, h] = o
                o_size[2 * (t >> 3) + bg] += o * o
            elif kind == "Q":
                q_wave((Q_STEADY if steady else Q_EARLY)[n], t, zero)
            elif kind in "ot":
                o_wave(n, t - (kind == "t"), zero, o_zero if last == "P" else zero, steady)
            elif kind == "x":
                slab = jnp.minimum(5 * (t - N_EARLY) + n // 4, 27)
                g = 2 + (slab >= 14).astype(jnp.int32)
                quarter = range(7 * (7 * (n % 4) // 4), 7 * (7 * (n % 4 + 1) // 4))
                row = pl.multiple_of(16 * (slab - 14 * (g - 2)), 16)
                x_slab(x_raw.at[g], x_ops.at[g], row, quarter if n < 16 else range(49))
            elif kind == "r":
                check_x(jnp.minimum(5 * (t - N_EARLY) + n, 55), o_zero)
            elif kind == "c":
                check_weights(n, t, o_zero)
            elif kind == "w":
                transfer(wait, 0, t, sorted(WHOLE) if steady else PIECEWISE[n], n)
            elif steady:
                for branch in range(2):
                    pl.when((t + 1) >> 3 == branch)(lambda: transfer(start, branch, t + 1, WHOLE[n:n + 1], 0))
                if n == 3:
                    pl.when(((t - 1) >> 1) & 3 == 3)(lambda: send(t - 1, 0, TB))
            else:
                pl.when(t + 1 < N_EARLY)(lambda: transfer(start, 0, t + 1, PIECEWISE[n], n))
                if n == 0:
                    pl.when(t + 1 == N_EARLY)(lambda: transfer(start, 0, N_EARLY, WHOLE, 0))

    x_copy(0, 0).start()
    for n, items in enumerate(PIECEWISE):

        @pl.loop(32 * n // len(PIECEWISE), 32 * (n + 1) // len(PIECEWISE))
        def _(i):
            carry[i >> 4, 0, (i >> 2) & 3, i & 3] = jnp.zeros((SQ, 128), f32)

        transfer(start, 0, 0, items, n)

    @pl.loop(0, 4)
    def _(n):
        o_size[n] = jnp.zeros((SQ, 128), f32)
        for row, rows, v in ((0, 8, math.inf), (8, 40, 0.0)):
            so_buf[0, TB + 1, n, pl.ds(row, rows)] = jnp.full((rows, 128), v, f32)

    q_size[...] = jnp.full(q_size.shape, math.inf, f32)
    x_copy(0, 1).start()

    @pl.loop(0, N_EARLY)
    def _(t):
        pl.when(t < 2)(lambda: x_operands(t))
        lax.cond(
            t == 0,
            lambda: run(False, EARLY_STEPS[:len(PLAN_FIRST)], t),
            lambda: run(False, NEXT_STEPS, t),
        )
        run(False, EARLY_STEPS[len(PLAN_FIRST):], t)

        @pl.when(t == N_EARLY - 2)
        def _():
            x_copy(1, 0).start()
            x_copy(1, 1).start()

    x_copy(1, 0).wait()
    x_copy(1, 1).wait()
    pl.loop(N_EARLY, NTILE)(functools.partial(run, True, STEADY_STEPS))

    finished = [
        max(n for n, w in enumerate(O_WAVES) for k, _ in w[1] if k[0] == "result" and k[1][1] // 2 == b)
        for b in range(TB)
    ]
    for n in range(len(O_WAVES)):
        if n >= N_IN_TILE:
            o_wave(n, NTILE - 1, 0, 0, True)
        for b in range(TB):
            if finished[b] == n:
                send(NTILE - 1, b, 1)
    sent(0)

    row_sums = lambda v: scores(jnp.ones((16, 128), bf16), v.astype(bf16))[:8]
    doubt, row_doubt = jnp.zeros((8, 128), f32), jnp.zeros((8, HALF), f32)
    for n in range(4):
        low, high, weight = (so_buf[0, TB + 1, n, pl.ds(8 * i, 8)] for i in range(3))
        doubt = jnp.where(_comparable(high, weight, W_HIGH_SPREAD), doubt, 1.0)
        doubt = jnp.where(_comparable(weight, low, W_LOW_SPREAD), doubt, 1.0)
        if n % 2 == 0:
            scale = jnp.max(so_buf[0, TB + 1, n, pl.ds(32, 16)], axis=0, keepdims=True) * weight
            doubt = jnp.where(_comparable(scale, q_size[n // 2], Q_SPREAD), doubt, 1.0)
            continue
        for g in (n - 1, n):
            scale = row_sums(o_size[g, :HALF] + o_size[g, HALF:]) * weight[:, :HALF] * (1 / (2 * TB))
            for b, r in itertools.product(range(TB), (0, HALF)):
                y = out_buf[g, 0, b, pl.ds(r, HALF)].astype(f32)
                row_doubt = jnp.where(_comparable(scale, row_sums(y * y), OUT_SPREAD), row_doubt, 1.0)
    redo = jnp.max(doubt) + jnp.max(row_doubt) > 0
    sent(1)
    pl.when(redo)(lambda: pl.loop(0, 2 * B)(plain))


@jax.jit
def pallas_concat_heads__gqa_block_cached__mha_block_cached__near_ridge_kernel(
    A_x: jax.Array,
    A_k_cache: jax.Array,
    A_v_cache: jax.Array,
    A_wq: jax.Array,
    A_wo: jax.Array,
    B_x: jax.Array,
    B_k_cache: jax.Array,
    B_v_cache: jax.Array,
    B_wq: jax.Array,
    B_wo: jax.Array,
):
    f32, bf16 = jnp.float32, jnp.bfloat16
    args = (A_x, A_k_cache, A_v_cache, A_wq, A_wo, B_x, B_k_cache, B_v_cache, B_wq, B_wo)
    shapes = [(B, SQ, D), (B, H, SK, DH), (B, H, SK, DH), (D, H * DH), (H * DH, D)] * 2
    assert [a.shape for a in args] == shapes and all(a.dtype == bf16 for a in args)
    return pl.pallas_call(
        _kernel,
        in_specs=[pl.BlockSpec(memory_space=pl.ANY)] * len(args),
        out_specs=pl.BlockSpec(memory_space=pl.ANY),
        out_shape=jax.ShapeDtypeStruct((B, SQ, 2 * D), bf16),
        scratch_shapes=[
            pltpu.VMEM((4, TB, SQ, D), bf16),
            pltpu.VMEM((4, 64, SQ, 128), bf16),
            pltpu.VMEM((2, TB, TH, SK, DH), bf16),
            pltpu.VMEM((2, D, TH * DH), bf16),
            pltpu.VMEM((2, 4, TH * DH, 128), bf16),
            pltpu.VMEM((2, TB, TH, SK, DH), bf16),
            pltpu.VMEM((1, TB, TH, SQ, DH), bf16),
            pltpu.VMEM((1, TB + 2, TH, SQ, 128), f32),
            pltpu.VMEM((1, 2, 4, SQ, 128), bf16),
            pltpu.VMEM((1, Q_SLOTS, SQ, 128), f32),
            pltpu.VMEM((1, O_SLOTS + O_SLOTS % 2, HALF, 128), f32),
            pltpu.VMEM((4, SQ, 128), f32),
            pltpu.VMEM((2, 5, TB, 4, SQ, 128), f32),
            pltpu.VMEM((4, 4, TB, SQ, 128), bf16),
            pltpu.VMEM((2, 8, 128), f32),
            pltpu.SemaphoreType.DMA((len(PIECEWISE),)),
            pltpu.SemaphoreType.DMA((4,)),
            pltpu.SemaphoreType.DMA((2,)),
        ],
        compiler_params=pltpu.CompilerParams(vmem_limit_bytes=100 * 2**20),
    )(*args)
```
